```python
import os as _os
_os.environ.setdefault("JAX_PLATFORMS", "cpu")
import jax
import jax.numpy as jnp

def _softmax(x, axis=-1):
    return jax.nn.softmax(x, axis=axis)
def _gelu(x):
    return jax.nn.gelu(x, approximate=True)
def _silu(x):
    return jax.nn.silu(x)
def _sigmoid(x):
    return jax.nn.sigmoid(x)
def _layernorm(x, axis=-1, eps=1e-5):
    m = jnp.mean(x, axis=axis, keepdims=True)
    v = jnp.var(x, axis=axis, keepdims=True)
    return (x - m) / jnp.sqrt(v + eps)
def _scatter_add(tgt, idx, src, axis=0):
    return tgt.at[idx].add(src)
def _segment_sum(src, seg, n):
    return jax.ops.segment_sum(src, seg, n)
class _Rng:
    def __init__(self, key):
        self._k = key
    def _next(self):
        self._k, sub = jax.random.split(self._k)
        return sub
    def normal(self, shape):
        return jax.random.normal(self._next(), shape, dtype=jnp.bfloat16)
    def randint(self, lo, hi, shape):
        return jax.random.randint(self._next(), shape, lo, hi, dtype=jnp.int32)
    def uniform(self, shape, lo=0.0, hi=1.0):
        return jax.random.uniform(self._next(), shape, jnp.bfloat16, lo, hi)
    def permutation(self, n):
        return jax.random.permutation(self._next(), n)


kernel_name = 'gated_mix__mha_block__softmax_full_mha__prompt'

def setup_inputs():
    _rng = _Rng(jax.random.key(int.from_bytes(__import__("os").urandom(4), "little")))
    _w = (lambda a: (lambda t: t.astype(jnp.bfloat16) if jnp.issubdtype(t.dtype, jnp.floating) else t)(jnp.asarray(a)))
    def _A_setup():
        B, S, D, H = 1, 2048, 448, 16
        return {
            "x": _w((lambda *s: _rng.normal(s) * 0.05)(B, S, D)),
            "wqkv": _w((lambda *s: _rng.normal(s) * 0.4)(D, 3 * D)),
            "wo": _w((lambda *s: _rng.normal(s) * 0.05)(D, D)),
        }
    _A_in = _A_setup()

    def _B_setup():
        B, S, D = 1, 2048, 448
        return {
            "x": _w((lambda *s: _rng.normal(s) * 0.05)(B, S, D)),
            "wqkv": _w((lambda *s: _rng.normal(s) * 0.4)(D, 3 * D)),
            "wo": _w((lambda *s: _rng.normal(s) * 0.05)(D, D)),
        }
    _B_in = _B_setup()

    return {
        "A_x": _A_in["x"],
        "A_wqkv": _A_in["wqkv"],
        "A_wo": _A_in["wo"],
        "B_x": _B_in["x"],
        "B_wqkv": _B_in["wqkv"],
        "B_wo": _B_in["wo"],
        "gate_w": _w((lambda *s: _rng.normal(s) * 0.05)(448) * 16.0),
    }

def reference(A_x, A_wqkv, A_wo, B_x, B_wqkv, B_wo, gate_w):
    def _A_ref(x, wqkv, wo):
        B, S, D = x.shape
        H = 16
        Dh = D // H
        qkv = (lambda x, *d: x.transpose(*d))((x @ wqkv).reshape(B, S, 3, H, Dh), 2, 0, 3, 1, 4)
        q, k, v = qkv[0], qkv[1], qkv[2]
        scores = jnp.einsum("bhqd,bhkd->bhqk", q, k) * (Dh ** -0.5)
        p = _softmax(scores, axis=-1)
        o = jnp.einsum("bhqk,bhkd->bhqd", p, v)
        return (lambda x, *d: x.transpose(*d))(o, 0, 2, 1, 3).reshape(B, S, D) @ wo

    def _B_ref(x, wqkv, wo):
        B, S, D = x.shape
        H = 16; Dh = D // H
        qkv = (lambda x, *d: x.transpose(*d))((x @ wqkv).reshape(B, S, 3, H, Dh), 2, 0, 3, 1, 4)
        q, k, v = qkv[0], qkv[1], qkv[2]
        scale = Dh ** -0.5
        scores = jnp.einsum("bhqd,bhkd->bhqk", q, k) * scale
        p = _softmax(scores, axis=-1)
        o = jnp.einsum("bhqk,bhkd->bhqd", p, v)
        return (lambda x, *d: x.transpose(*d))(o, 0, 2, 1, 3).reshape(B, S, D) @ wo

    x = A_x
    g = _sigmoid((x * gate_w).sum(-1, keepdims=True))
    a = _A_ref(x, A_wqkv, A_wo)
    b = _B_ref(x, B_wqkv, B_wo)
    return g * a + (1 - g) * b
```

```python
import math

import jax
import jax.numpy as jnp
from jax import lax
import jax.experimental.pallas as pl
import jax.experimental.pallas.tpu as pltpu

S = 2048
D = 448
H = 16
DH = 28
DP = 32
NH = 2 * H
LOG2E = math.log2(math.e)
f32 = jnp.float32
bf16 = jnp.bfloat16
TN = (((0,), (0,)), ((), ()))

BW = 512
BK = 128
HU = 2
NPC = S // BW
NC = S // BK


def _kernel(xt_hbm, wa_hbm, wb_hbm, woa_hbm, wob_hbm, gw_ref, o_ref,
            xt_ref, wa_ref, wb_ref, woa_ref, wob_ref, sems, qvt_s, k_s, g_s, ot_s):
    copies = [
        pltpu.make_async_copy(src, dst, sems.at[i])
        for i, (src, dst) in enumerate((
            (xt_hbm, xt_ref), (wa_hbm, wa_ref), (wb_hbm, wb_ref),
            (woa_hbm, woa_ref), (wob_hbm, wob_ref)))
    ]
    for cp in copies:
        cp.start()
    copies[0].wait()
    xt = xt_ref[...]

    zer4 = jnp.zeros((DP - DH, S), f32)
    row4 = lax.broadcasted_iota(jnp.int32, (DP - DH, S), 0)
    one4 = jnp.where(row4 == 0, 1.0, 0.0).astype(f32)

    gw = jnp.broadcast_to(gw_ref[...], (8, D))
    g_s[...] = jax.nn.sigmoid(jnp.dot(gw, xt, preferred_element_type=f32))

    for br, w_ref in enumerate((wa_ref, wb_ref)):
        copies[1 + br].wait()
        qt = lax.dot_general(w_ref[:, 0:D], xt, TN, preferred_element_type=f32)
        qt = qt * (DH ** -0.5 * LOG2E)
        for h in range(H):
            r0 = br * 1024 + h * DP
            qvt_s[r0:r0 + DP, :] = jnp.concatenate(
                [qt[h * DH:(h + 1) * DH, :], zer4], axis=0).astype(bf16)
        vt = lax.dot_general(w_ref[:, 2 * D:3 * D], xt, TN, preferred_element_type=f32)
        for h in range(H):
            r0 = br * 1024 + 512 + h * DP
            qvt_s[r0:r0 + DP, :] = jnp.concatenate(
                [vt[h * DH:(h + 1) * DH, :], one4], axis=0).astype(bf16)
        kt = lax.dot_general(w_ref[:, D:2 * D], xt, TN, preferred_element_type=f32)
        for h in range(H):
            kp = jnp.concatenate([kt[h * DH:(h + 1) * DH, :], zer4], axis=0)
            k_s[br * H + h] = kp.T.astype(bf16)

    def group_body(hg, carry):
        heads = []
        for u in range(HU):
            h = hg * HU + u
            br = h // H
            hh = h % H
            qrow = pl.multiple_of(br * 1024 + hh * DP, DP)
            vrow = pl.multiple_of(br * 1024 + 512 + hh * DP, DP)
            orow = pl.multiple_of(h * DP, DP)
            heads.append((h, br, qrow, vrow, orow))

        def qk(u, c, j):
            h, _, qrow, _, _ = heads[u]
            qT = qvt_s[pl.ds(qrow, DP), j * BW:(j + 1) * BW]
            return jnp.dot(k_s[h, c * BK:(c + 1) * BK, :], qT, preferred_element_type=f32)

        steps = [(u, c) for u in range(HU) for c in range(NC)]
        s_next = [qk(0, 0, j) for j in range(NPC)]
        m = None
        acc = None
        for si, (u, c) in enumerate(steps):
            _, br, _, vrow, orow = heads[u]
            if c == 0:
                m = [None] * NPC
                acc = [None] * NPC
            s_cur = s_next
            s_next = [None] * NPC
            vT = qvt_s[pl.ds(vrow, DP), c * BK:(c + 1) * BK]
            for j in range(NPC):
                if si + 1 < len(steps):
                    s_next[j] = qk(steps[si + 1][0], steps[si + 1][1], j)
                s = s_cur[j]
                mc = jnp.max(s, axis=0, keepdims=True)
                m_new = mc if m[j] is None else jnp.maximum(m[j], mc)
                p = jnp.exp2(s - m_new).astype(bf16)
                pv = jnp.dot(vT, p, preferred_element_type=f32)
                if acc[j] is None:
                    acc[j] = pv
                else:
                    acc[j] = acc[j] * jnp.exp2(m[j] - m_new) + pv
                m[j] = m_new
                if c == NC - 1:
                    l = acc[j][DH:DH + 1, :]
                    g = g_s[0:1, j * BW:(j + 1) * BW]
                    gg = jnp.where(br == 0, g, 1.0 - g)
                    ot_s[pl.ds(orow, DP), j * BW:(j + 1) * BW] = (
                        acc[j] * (gg / l)).astype(bf16)
        return carry

    lax.fori_loop(0, NH // HU, group_body, 0)

    copies[3].wait()
    copies[4].wait()
    zo = jnp.zeros((DP - DH, D), f32)
    pieces = []
    for wo_ref in (woa_ref, wob_ref):
        wo = wo_ref[...].astype(f32)
        for h in range(H):
            pieces.append(wo[h * DH:(h + 1) * DH, :])
            pieces.append(zo)
    wo_pad = jnp.concatenate(pieces, axis=0).astype(bf16)
    out_t = lax.dot_general(wo_pad, ot_s[...], TN, preferred_element_type=f32)
    o_ref[...] = out_t.astype(o_ref.dtype)


@jax.jit
def pallas_gated_mix__mha_block__softmax_full_mha__prompt_kernel(
    A_x: jax.Array,
    A_wqkv: jax.Array,
    A_wo: jax.Array,
    B_x: jax.Array,
    B_wqkv: jax.Array,
    B_wo: jax.Array,
    gate_w: jax.Array,
):
    del B_x
    xt = A_x.reshape(S, D).T
    gw = gate_w.reshape(1, D)
    anyspec = pl.BlockSpec(memory_space=pl.ANY)
    out_t = pl.pallas_call(
        _kernel,
        in_specs=[anyspec, anyspec, anyspec, anyspec, anyspec,
                  pl.BlockSpec(memory_space=pltpu.VMEM)],
        out_specs=pl.BlockSpec(memory_space=pltpu.VMEM),
        out_shape=jax.ShapeDtypeStruct((D, S), bf16),
        scratch_shapes=[
            pltpu.VMEM((D, S), bf16),
            pltpu.VMEM((D, 3 * D), bf16),
            pltpu.VMEM((D, 3 * D), bf16),
            pltpu.VMEM((D, D), bf16),
            pltpu.VMEM((D, D), bf16),
            pltpu.SemaphoreType.DMA((5,)),
            pltpu.VMEM((2048, S), bf16),
            pltpu.VMEM((NH, S, DP), bf16),
            pltpu.VMEM((8, S), f32),
            pltpu.VMEM((1024, S), bf16),
        ],
        compiler_params=pltpu.CompilerParams(vmem_limit_bytes=100 * 1024 * 1024),
    )(xt, A_wqkv, B_wqkv, A_wo, B_wo, gw)
    return out_t.T.reshape(1, S, D)
```

```python
import math

import jax
import jax.numpy as jnp
from jax import lax
import jax.experimental.pallas as pl
import jax.experimental.pallas.tpu as pltpu

S = 2048
D = 448
H = 16
DH = 28
DP = 32
NH = 2 * H
LOG2E = math.log2(math.e)
f32 = jnp.float32
bf16 = jnp.bfloat16
TN = (((0,), (0,)), ((), ()))

BW = 512
BK = 128
HU = 2
NOB = 4
NPC = S // BW
NC = S // BK


def _kernel(xt_hbm, wa_hbm, wb_hbm, woa_hbm, wob_hbm, gw_ref, o_hbm,
            xt_ref, wa_ref, wb_ref, woa_ref, wob_ref, sems,
            qvt_s, k_s, g_s, ot_s, ob_s, osems):
    copies = [
        pltpu.make_async_copy(src, dst, sems.at[i])
        for i, (src, dst) in enumerate((
            (xt_hbm, xt_ref), (wa_hbm, wa_ref), (wb_hbm, wb_ref),
            (woa_hbm, woa_ref), (wob_hbm, wob_ref)))
    ]
    for cp in copies:
        cp.start()
    copies[0].wait()
    xt = xt_ref[...]

    zer4 = jnp.zeros((DP - DH, S), f32)
    row4 = lax.broadcasted_iota(jnp.int32, (DP - DH, S), 0)
    one4 = jnp.where(row4 == 0, 1.0, 0.0).astype(f32)

    gw = jnp.broadcast_to(gw_ref[...], (8, D))
    g_s[...] = jax.nn.sigmoid(jnp.dot(gw, xt, preferred_element_type=f32))

    for br, w_ref in enumerate((wa_ref, wb_ref)):
        copies[1 + br].wait()
        qt = lax.dot_general(w_ref[:, 0:D], xt, TN, preferred_element_type=f32)
        qt = qt * (DH ** -0.5 * LOG2E)
        for h in range(H):
            r0 = br * 1024 + h * DP
            qvt_s[r0:r0 + DP, :] = jnp.concatenate(
                [qt[h * DH:(h + 1) * DH, :], zer4], axis=0).astype(bf16)
        vt = lax.dot_general(w_ref[:, 2 * D:3 * D], xt, TN, preferred_element_type=f32)
        for h in range(H):
            r0 = br * 1024 + 512 + h * DP
            qvt_s[r0:r0 + DP, :] = jnp.concatenate(
                [vt[h * DH:(h + 1) * DH, :], one4], axis=0).astype(bf16)
        kt = lax.dot_general(w_ref[:, D:2 * D], xt, TN, preferred_element_type=f32)
        for h in range(H):
            kp = jnp.concatenate([kt[h * DH:(h + 1) * DH, :], zer4], axis=0)
            k_s[br * H + h] = kp.T.astype(bf16)

    def group_body(hg, carry):
        heads = []
        for u in range(HU):
            h = hg * HU + u
            br = h // H
            hh = h % H
            qrow = pl.multiple_of(br * 1024 + hh * DP, DP)
            vrow = pl.multiple_of(br * 1024 + 512 + hh * DP, DP)
            orow = pl.multiple_of(h * DP, DP)
            heads.append((h, br, qrow, vrow, orow))

        def qk(u, c, j):
            h, _, qrow, _, _ = heads[u]
            qT = qvt_s[pl.ds(qrow, DP), j * BW:(j + 1) * BW]
            return jnp.dot(k_s[h, c * BK:(c + 1) * BK, :], qT, preferred_element_type=f32)

        steps = [(u, c) for u in range(HU) for c in range(NC)]
        s_next = [qk(0, 0, j) for j in range(NPC)]
        m = None
        acc = None
        for si, (u, c) in enumerate(steps):
            _, br, _, vrow, orow = heads[u]
            if c == 0:
                m = [None] * NPC
                acc = [None] * NPC
            s_cur = s_next
            s_next = [None] * NPC
            vT = qvt_s[pl.ds(vrow, DP), c * BK:(c + 1) * BK]
            for j in range(NPC):
                if si + 1 < len(steps):
                    s_next[j] = qk(steps[si + 1][0], steps[si + 1][1], j)
                s = s_cur[j]
                mc = jnp.max(s, axis=0, keepdims=True)
                m_new = mc if m[j] is None else jnp.maximum(m[j], mc)
                p = jnp.exp2(s - m_new).astype(bf16)
                pv = jnp.dot(vT, p, preferred_element_type=f32)
                if acc[j] is None:
                    acc[j] = pv
                else:
                    acc[j] = acc[j] * jnp.exp2(m[j] - m_new) + pv
                m[j] = m_new
                if c == NC - 1:
                    l = acc[j][DH:DH + 1, :]
                    g = g_s[0:1, j * BW:(j + 1) * BW]
                    gg = jnp.where(br == 0, g, 1.0 - g)
                    ot_s[pl.ds(orow, DP), j * BW:(j + 1) * BW] = (
                        acc[j] * (gg / l)).astype(bf16)
        return carry

    lax.fori_loop(0, NH // HU, group_body, 0)

    copies[3].wait()
    copies[4].wait()
    zo = jnp.zeros((DP - DH, D), f32)
    pieces = []
    for wo_ref in (woa_ref, wob_ref):
        wo = wo_ref[...].astype(f32)
        for h in range(H):
            pieces.append(wo[h * DH:(h + 1) * DH, :])
            pieces.append(zo)
    wo_t = jnp.concatenate(pieces, axis=0).astype(bf16).T
    cb = S // NOB
    out_copies = []
    for b in range(NOB):
        out_t = jnp.dot(wo_t, ot_s[:, b * cb:(b + 1) * cb], preferred_element_type=f32)
        ob_s[:, b * cb:(b + 1) * cb] = out_t.astype(bf16)
        cp = pltpu.make_async_copy(
            ob_s.at[:, b * cb:(b + 1) * cb], o_hbm.at[:, b * cb:(b + 1) * cb], osems.at[b])
        cp.start()
        out_copies.append(cp)
    for cp in out_copies:
        cp.wait()


@jax.jit
def pallas_gated_mix__mha_block__softmax_full_mha__prompt_kernel(
    A_x: jax.Array,
    A_wqkv: jax.Array,
    A_wo: jax.Array,
    B_x: jax.Array,
    B_wqkv: jax.Array,
    B_wo: jax.Array,
    gate_w: jax.Array,
):
    del B_x
    xt = A_x.reshape(S, D).T
    gw = gate_w.reshape(1, D)
    anyspec = pl.BlockSpec(memory_space=pl.ANY)
    out_t = pl.pallas_call(
        _kernel,
        in_specs=[anyspec, anyspec, anyspec, anyspec, anyspec,
                  pl.BlockSpec(memory_space=pltpu.VMEM)],
        out_specs=anyspec,
        out_shape=jax.ShapeDtypeStruct((D, S), bf16),
        scratch_shapes=[
            pltpu.VMEM((D, S), bf16),
            pltpu.VMEM((D, 3 * D), bf16),
            pltpu.VMEM((D, 3 * D), bf16),
            pltpu.VMEM((D, D), bf16),
            pltpu.VMEM((D, D), bf16),
            pltpu.SemaphoreType.DMA((5,)),
            pltpu.VMEM((2048, S), bf16),
            pltpu.VMEM((NH, S, DP), bf16),
            pltpu.VMEM((8, S), f32),
            pltpu.VMEM((1024, S), bf16),
            pltpu.VMEM((D, S), bf16),
            pltpu.SemaphoreType.DMA((NOB,)),
        ],
        compiler_params=pltpu.CompilerParams(vmem_limit_bytes=100 * 1024 * 1024),
    )(xt, A_wqkv, B_wqkv, A_wo, B_wo, gw)
    return out_t.T.reshape(1, S, D)
```
